```python
import os as _os
_os.environ.setdefault("JAX_PLATFORMS", "cpu")
import jax
import jax.numpy as jnp

def _softmax(x, axis=-1):
    return jax.nn.softmax(x, axis=axis)
def _gelu(x):
    return jax.nn.gelu(x, approximate=True)
def _silu(x):
    return jax.nn.silu(x)
def _sigmoid(x):
    return jax.nn.sigmoid(x)
def _layernorm(x, axis=-1, eps=1e-5):
    m = jnp.mean(x, axis=axis, keepdims=True)
    v = jnp.var(x, axis=axis, keepdims=True)
    return (x - m) / jnp.sqrt(v + eps)
def _scatter_add(tgt, idx, src, axis=0):
    return tgt.at[idx].add(src)
def _segment_sum(src, seg, n):
    return jax.ops.segment_sum(src, seg, n)
class _Rng:
    def __init__(self, key):
        self._k = key
    def _next(self):
        self._k, sub = jax.random.split(self._k)
        return sub
    def normal(self, shape):
        return jax.random.normal(self._next(), shape, dtype=jnp.bfloat16)
    def randint(self, lo, hi, shape):
        return jax.random.randint(self._next(), shape, lo, hi, dtype=jnp.int32)
    def uniform(self, shape, lo=0.0, hi=1.0):
        return jax.random.uniform(self._next(), shape, jnp.bfloat16, lo, hi)
    def permutation(self, n):
        return jax.random.permutation(self._next(), n)


kernel_name = 'standalone__mha_softmax__near_ridge'

def setup_inputs():
    _rng = _Rng(jax.random.key(int.from_bytes(__import__("os").urandom(4), "little")))
    _w = (lambda a: (lambda t: t.astype(jnp.bfloat16) if jnp.issubdtype(t.dtype, jnp.floating) else t)(jnp.asarray(a)))
    B, H, Sq, Sk, D = 8, 16, 192, 1024, 256
    return {
        "q": _w((lambda *s: _rng.normal(s) * 0.4)(B, H, Sq, D)),
        "k": _w((lambda *s: _rng.normal(s) * 0.4)(B, H, Sk, D)),
        "v": _w((lambda *s: _rng.normal(s) * 0.05)(B, H, Sk, D)),
    }

def reference(q, k, v):
    scale = q.shape[-1] ** -0.5
    scores = jnp.einsum("bhqd,bhkd->bhqk", q, k) * scale
    p = _softmax(scores, axis=-1)
    return jnp.einsum("bhqk,bhkd->bhqd", p, v)
```

```python
import math

import jax
import jax.numpy as jnp
from jax import lax
import jax.experimental.pallas as pl
import jax.experimental.pallas.tpu as pltpu

_HB = 2


def _attn_kernel(q_ref, k_ref, v_ref, o_ref):
    d = q_ref.shape[-1]
    c = (d ** -0.5) * math.log2(math.e)
    for h in range(_HB):
        q = q_ref[h]
        k = k_ref[h]
        v = v_ref[h]
        s = lax.dot_general(q, k, (((1,), (1,)), ((), ())),
                            preferred_element_type=jnp.float32)
        m = jnp.max(s, axis=-1, keepdims=True)
        p = jnp.exp2((s - m) * c)
        l = jnp.sum(p, axis=-1, keepdims=True)
        o = jnp.dot(p.astype(jnp.bfloat16), v, preferred_element_type=jnp.float32)
        o_ref[h] = (o * pl.reciprocal(l, approx=False)).astype(o_ref.dtype)


@jax.jit
def pallas_standalone__mha_softmax__near_ridge_kernel(
    q: jax.Array,
    k: jax.Array,
    v: jax.Array,
):
    B, H, Sq, D = q.shape
    Sk = k.shape[2]
    BH = B * H
    q3 = q.reshape(BH, Sq, D)
    k3 = k.reshape(BH, Sk, D)
    v3 = v.reshape(BH, Sk, D)
    out = pl.pallas_call(
        _attn_kernel,
        grid=(BH // _HB,),
        in_specs=[
            pl.BlockSpec((_HB, Sq, D), lambda i: (i, 0, 0)),
            pl.BlockSpec((_HB, Sk, D), lambda i: (i, 0, 0)),
            pl.BlockSpec((_HB, Sk, D), lambda i: (i, 0, 0)),
        ],
        out_specs=pl.BlockSpec((_HB, Sq, D), lambda i: (i, 0, 0)),
        out_shape=jax.ShapeDtypeStruct((BH, Sq, D), q.dtype),
        compiler_params=pltpu.CompilerParams(
            dimension_semantics=("arbitrary",),
            vmem_limit_bytes=64 * 1024 * 1024,
        ),
    )(q3, k3, v3)
    return out.reshape(B, H, Sq, D)
```

```python
import math

import jax
import jax.numpy as jnp
from jax import lax
import jax.experimental.pallas as pl
import jax.experimental.pallas.tpu as pltpu

_NBUF = 3
_QCHUNK = 16
_WLEAD = 2
_WROWS = 64


def _make_kernel(B, H, Sq, Sk, D):
    n = B * H
    nq = n // _QCHUNK
    rows = H * Sq
    n_w = rows // _WROWS
    n_early = (rows - _WLEAD * Sq) // _WROWS
    c = (D ** -0.5) * math.log2(math.e)

    def kernel(q_hbm, k_hbm, v_hbm, o_hbm, qb, kb, vb, ob, sq, sk, sv, so):
        def k_copy(i, slot):
            return pltpu.make_async_copy(k_hbm.at[i], kb.at[slot], sk.at[slot])

        def v_copy(i, slot):
            return pltpu.make_async_copy(v_hbm.at[i], vb.at[slot], sv.at[slot])

        def q_copy(j):
            return pltpu.make_async_copy(
                q_hbm.at[pl.ds(j * _QCHUNK, _QCHUNK)], qb.at[j % 2], sq.at[j % 2])

        def out_copy(j):
            sl = pl.ds(j * _WROWS, _WROWS)
            return pltpu.make_async_copy(ob.at[:, sl], o_hbm.at[:, sl], so.at[j])

        k_copy(0, 0).start()
        q_copy(0).start()
        v_copy(0, 0).start()
        for j in range(1, _NBUF - 1):
            k_copy(j, j).start()
            v_copy(j, j).start()

        def body(i, carry):
            slot = i % _NBUF
            nxt = i + (_NBUF - 1)

            @pl.when(nxt < n)
            def _():
                k_copy(nxt, nxt % _NBUF).start()
                v_copy(nxt, nxt % _NBUF).start()

            j = i // _QCHUNK

            @pl.when(i % _QCHUNK == 0)
            def _():
                q_copy(j).wait()

                @pl.when(j + 1 < nq)
                def _():
                    q_copy(j + 1).start()

            k_copy(i, slot).wait()
            v_copy(i, slot).wait()

            @pl.when(i == n - _WLEAD)
            def _():
                for w in range(n_early):
                    out_copy(w).start()

            q = qb[j % 2, i % _QCHUNK]
            s = lax.dot_general(q, kb[slot], (((1,), (1,)), ((), ())),
                                preferred_element_type=jnp.float32)
            m = jnp.max(s, axis=-1, keepdims=True)
            p = jnp.exp2((s - m) * c)
            l = jnp.sum(p, axis=-1, keepdims=True)
            o = jnp.dot(p.astype(vb.dtype), vb[slot],
                        preferred_element_type=jnp.float32)
            o = o * pl.reciprocal(l, approx=False)
            r0 = pl.multiple_of((i % H) * Sq, Sq)
            ob[i // H, pl.ds(r0, Sq), :] = o.astype(ob.dtype)
            return carry

        lax.fori_loop(0, n, body, 0)

        for w in range(n_early, n_w):
            out_copy(w).start()
        for w in range(n_w):
            out_copy(w).wait()

    return kernel, n_w


@jax.jit
def pallas_standalone__mha_softmax__near_ridge_kernel(
    q: jax.Array,
    k: jax.Array,
    v: jax.Array,
):
    B, H, Sq, D = q.shape
    Sk = k.shape[2]
    n = B * H
    assert n % _QCHUNK == 0 and Sq % _WROWS == 0 and H >= _WLEAD and n >= _NBUF
    kernel, n_w = _make_kernel(B, H, Sq, Sk, D)
    out = pl.pallas_call(
        kernel,
        in_specs=[pl.BlockSpec(memory_space=pl.ANY)] * 3,
        out_specs=pl.BlockSpec(memory_space=pl.ANY),
        out_shape=jax.ShapeDtypeStruct((B, H * Sq, D), q.dtype),
        scratch_shapes=[
            pltpu.VMEM((2, _QCHUNK, Sq, D), q.dtype),
            pltpu.VMEM((_NBUF, Sk, D), k.dtype),
            pltpu.VMEM((_NBUF, Sk, D), v.dtype),
            pltpu.VMEM((B, H * Sq, D), q.dtype),
            pltpu.SemaphoreType.DMA((2,)),
            pltpu.SemaphoreType.DMA((_NBUF,)),
            pltpu.SemaphoreType.DMA((_NBUF,)),
            pltpu.SemaphoreType.DMA((n_w,)),
        ],
        compiler_params=pltpu.CompilerParams(
            vmem_limit_bytes=64 * 1024 * 1024,
        ),
    )(q.reshape(n, Sq, D), k.reshape(n, Sk, D), v.reshape(n, Sk, D))
    return out.reshape(B, H, Sq, D)
```

```python
import functools
import math

import jax
import jax.numpy as jnp
from jax import lax
import jax.experimental.pallas as pl
import jax.experimental.pallas.tpu as pltpu

_NBUF = 4
_QCHUNK = 16
_WROWS = 64


def _attention(q, k, v):
    c = (q.shape[-1] ** -0.5) * math.log2(math.e)
    s = lax.dot_general(q, k, (((1,), (1,)), ((), ())),
                        preferred_element_type=jnp.float32)
    m = jnp.max(s, axis=-1, keepdims=True)
    p = jnp.exp2((s - m) * c)
    l = jnp.sum(p, axis=-1, keepdims=True)
    o = jnp.dot(p.astype(v.dtype), v, preferred_element_type=jnp.float32)
    return o * pl.reciprocal(l, approx=False)


def _stream(q_hbm, k_hbm, v_hbm, o_hbm, qb, kb, vb, ob, so, sq, sk, sv, *, heads):
    n, sq_len, _ = q_hbm.shape
    nq = n // _QCHUNK
    n_w = ob.shape[1] // _WROWS
    n_early = (ob.shape[1] - 2 * sq_len) // _WROWS

    def k_copy(i):
        slot = i % _NBUF
        return pltpu.make_async_copy(k_hbm.at[i], kb.at[slot], sk.at[slot])

    def v_copy(i):
        slot = i % _NBUF
        return pltpu.make_async_copy(v_hbm.at[i], vb.at[slot], sv.at[slot])

    def q_copy(j):
        return pltpu.make_async_copy(
            q_hbm.at[pl.ds(j * _QCHUNK, _QCHUNK)], qb.at[j % 2], sq.at[j % 2])

    def out_copy(w):
        rows = pl.ds(w * _WROWS, _WROWS)
        return pltpu.make_async_copy(ob.at[:, rows], o_hbm.at[:, rows], so.at[0])

    k_copy(0).start()
    q_copy(0).start()
    v_copy(0).start()
    for i in range(1, _NBUF - 1):
        k_copy(i).start()
        v_copy(i).start()

    def body(i, carry):
        nxt = i + (_NBUF - 1)

        @pl.when(nxt < n)
        def _():
            k_copy(nxt).start()
            v_copy(nxt).start()

        j = i // _QCHUNK

        @pl.when(i % _QCHUNK == 0)
        def _():
            q_copy(j).wait()

            @pl.when(j + 1 < nq)
            def _():
                q_copy(j + 1).start()

        @pl.when(i < n - 1)
        def _():
            k_copy(i).wait()

        v_copy(i).wait()

        @pl.when(i == n - 2)
        def _():
            k_copy(n - 1).wait()
            for w in range(n_early):
                out_copy(w).start()

        slot = i % _NBUF
        o = _attention(qb[j % 2, i % _QCHUNK], kb[slot], vb[slot])
        r0 = pl.multiple_of((i % heads) * sq_len, sq_len)
        ob[i // heads, pl.ds(r0, sq_len), :] = o.astype(ob.dtype)
        return carry

    lax.fori_loop(0, n, body, 0)

    for w in range(n_early, n_w):
        out_copy(w).start()


def _kernel(q_hbm, k_hbm, v_hbm, o_hbm, qb, kb, vb, ob, so, *, heads):
    pl.run_scoped(
        functools.partial(_stream, q_hbm, k_hbm, v_hbm, o_hbm, qb, kb, vb, ob, so,
                          heads=heads),
        pltpu.SemaphoreType.DMA((2,)),
        pltpu.SemaphoreType.DMA((_NBUF,)),
        pltpu.SemaphoreType.DMA((_NBUF,)),
    )
    pltpu.make_async_copy(ob, o_hbm, so.at[0]).wait()


@jax.jit
def pallas_standalone__mha_softmax__near_ridge_kernel(
    q: jax.Array,
    k: jax.Array,
    v: jax.Array,
):
    B, H, Sq, D = q.shape
    Sk = k.shape[2]
    n = B * H
    assert n % _QCHUNK == 0 and Sq % _WROWS == 0 and H >= 2 and n >= _NBUF >= 3
    out = pl.pallas_call(
        functools.partial(_kernel, heads=H),
        in_specs=[pl.BlockSpec(memory_space=pl.ANY)] * 3,
        out_specs=pl.BlockSpec(memory_space=pl.ANY),
        out_shape=jax.ShapeDtypeStruct((B, H * Sq, D), q.dtype),
        scratch_shapes=[
            pltpu.VMEM((2, _QCHUNK, Sq, D), q.dtype),
            pltpu.VMEM((_NBUF, Sk, D), k.dtype),
            pltpu.VMEM((_NBUF, Sk, D), v.dtype),
            pltpu.VMEM((B, H * Sq, D), q.dtype),
            pltpu.SemaphoreType.DMA((1,)),
        ],
        compiler_params=pltpu.CompilerParams(
            vmem_limit_bytes=64 * 1024 * 1024,
        ),
    )(q.reshape(n, Sq, D), k.reshape(n, Sk, D), v.reshape(n, Sk, D))
    return out.reshape(B, H, Sq, D)
```

```python
import functools
import math

import jax
import jax.numpy as jnp
from jax import lax
import jax.experimental.pallas as pl
import jax.experimental.pallas.tpu as pltpu

_HB = 2
_NGRP = 4
_NBUF = _HB * _NGRP
_QCHUNK = 16
_WROWS = 64


def _attention(q, k, v):
    c = (q.shape[-1] ** -0.5) * math.log2(math.e)
    s = lax.dot_general(q, k, (((1,), (1,)), ((), ())),
                        preferred_element_type=jnp.float32)
    s = s.astype(q.dtype).astype(jnp.float32)
    m = jnp.max(s, axis=-1, keepdims=True)
    p = jnp.exp2((s - m) * c)
    l = jnp.sum(p, axis=-1, keepdims=True)
    o = jnp.dot(p.astype(v.dtype), v, preferred_element_type=jnp.float32)
    return o * pl.reciprocal(l, approx=False)


def _stream(q_hbm, k_hbm, v_hbm, o_hbm, qb, kb, vb, ob, so, sq, sk, sv, *, heads):
    n, sq_len, _ = q_hbm.shape
    nt = n // _HB
    nq = n // _QCHUNK
    n_w = ob.shape[1] // _WROWS
    n_early = (ob.shape[1] - 2 * _HB * sq_len) // _WROWS

    def k_copy(i):
        slot = i % _NBUF
        return pltpu.make_async_copy(k_hbm.at[i], kb.at[slot], sk.at[slot])

    def v_copy(i):
        slot = i % _NBUF
        return pltpu.make_async_copy(v_hbm.at[i], vb.at[slot], sv.at[slot])

    def q_copy(j):
        return pltpu.make_async_copy(
            q_hbm.at[pl.ds(j * _QCHUNK, _QCHUNK)], qb.at[j % 2], sq.at[j % 2])

    def out_copy(w):
        rows = pl.ds(w * _WROWS, _WROWS)
        return pltpu.make_async_copy(ob.at[:, rows], o_hbm.at[:, rows], so.at[0])

    def wait_all_but_last_v(i0):
        for h in range(_HB):
            k_copy(i0 + h).wait()
            if h < _HB - 1:
                v_copy(i0 + h).wait()

    k_copy(0).start()
    q_copy(0).start()
    v_copy(0).start()
    for i in range(1, _NBUF - _HB):
        k_copy(i).start()
        v_copy(i).start()

    def body(t, carry):
        i0 = t * _HB
        nxt = i0 + (_NBUF - _HB)

        @pl.when(nxt < n)
        def _():
            for h in range(_HB):
                k_copy(nxt + h).start()
                v_copy(nxt + h).start()

        j = i0 // _QCHUNK

        @pl.when(i0 % _QCHUNK == 0)
        def _():
            q_copy(j).wait()

            @pl.when(j + 1 < nq)
            def _():
                q_copy(j + 1).start()

        @pl.when(t < nt - 1)
        def _():
            wait_all_but_last_v(i0)

        v_copy(i0 + _HB - 1).wait()

        @pl.when(t == nt - 2)
        def _():
            wait_all_but_last_v(n - _HB)
            for w in range(n_early):
                out_copy(w).start()

        for h in range(_HB):
            i = i0 + h
            slot = (t % _NGRP) * _HB + h
            o = _attention(qb[j % 2, i % _QCHUNK], kb[slot], vb[slot])
            r0 = pl.multiple_of((i % heads) * sq_len, sq_len)
            ob[i // heads, pl.ds(r0, sq_len), :] = o.astype(ob.dtype)
        return carry

    lax.fori_loop(0, nt, body, 0)

    for w in range(n_early, n_w):
        out_copy(w).start()


def _kernel(q_hbm, k_hbm, v_hbm, o_hbm, qb, kb, vb, ob, so, *, heads):
    pl.run_scoped(
        functools.partial(_stream, q_hbm, k_hbm, v_hbm, o_hbm, qb, kb, vb, ob, so,
                          heads=heads),
        pltpu.SemaphoreType.DMA((2,)),
        pltpu.SemaphoreType.DMA((_NBUF,)),
        pltpu.SemaphoreType.DMA((_NBUF,)),
    )
    pltpu.make_async_copy(ob, o_hbm, so.at[0]).wait()


@jax.jit
def pallas_standalone__mha_softmax__near_ridge_kernel(
    q: jax.Array,
    k: jax.Array,
    v: jax.Array,
):
    B, H, Sq, D = q.shape
    Sk = k.shape[2]
    n = B * H
    assert n % _QCHUNK == 0 and _QCHUNK % _HB == 0 and Sq % _WROWS == 0
    assert H >= 2 * _HB and n >= _NBUF and _NGRP >= 2
    out = pl.pallas_call(
        functools.partial(_kernel, heads=H),
        in_specs=[pl.BlockSpec(memory_space=pl.ANY)] * 3,
        out_specs=pl.BlockSpec(memory_space=pl.ANY),
        out_shape=jax.ShapeDtypeStruct((B, H * Sq, D), q.dtype),
        scratch_shapes=[
            pltpu.VMEM((2, _QCHUNK, Sq, D), q.dtype),
            pltpu.VMEM((_NBUF, Sk, D), k.dtype),
            pltpu.VMEM((_NBUF, Sk, D), v.dtype),
            pltpu.VMEM((B, H * Sq, D), q.dtype),
            pltpu.SemaphoreType.DMA((1,)),
        ],
        compiler_params=pltpu.CompilerParams(
            vmem_limit_bytes=64 * 1024 * 1024,
        ),
    )(q.reshape(n, Sq, D), k.reshape(n, Sk, D), v.reshape(n, Sk, D))
    return out.reshape(B, H, Sq, D)
```
